```python
import os as _os
_os.environ.setdefault("JAX_PLATFORMS", "cpu")
import jax
import jax.numpy as jnp

def _softmax(x, axis=-1):
    return jax.nn.softmax(x, axis=axis)
def _gelu(x):
    return jax.nn.gelu(x, approximate=True)
def _silu(x):
    return jax.nn.silu(x)
def _sigmoid(x):
    return jax.nn.sigmoid(x)
def _layernorm(x, axis=-1, eps=1e-5):
    m = jnp.mean(x, axis=axis, keepdims=True)
    v = jnp.var(x, axis=axis, keepdims=True)
    return (x - m) / jnp.sqrt(v + eps)
def _scatter_add(tgt, idx, src, axis=0):
    return tgt.at[idx].add(src)
def _segment_sum(src, seg, n):
    return jax.ops.segment_sum(src, seg, n)
class _Rng:
    def __init__(self, key):
        self._k = key
    def _next(self):
        self._k, sub = jax.random.split(self._k)
        return sub
    def normal(self, shape):
        return jax.random.normal(self._next(), shape, dtype=jnp.bfloat16)
    def randint(self, lo, hi, shape):
        return jax.random.randint(self._next(), shape, lo, hi, dtype=jnp.int32)
    def uniform(self, shape, lo=0.0, hi=1.0):
        return jax.random.uniform(self._next(), shape, jnp.bfloat16, lo, hi)
    def permutation(self, n):
        return jax.random.permutation(self._next(), n)


kernel_name = 'gated_mix__grouped_kv_mqa__glu_gated_reglu__prompt'

def setup_inputs():
    _rng = _Rng(jax.random.key(int.from_bytes(__import__("os").urandom(4), "little")))
    _w = (lambda a: (lambda t: t.astype(jnp.bfloat16) if jnp.issubdtype(t.dtype, jnp.floating) else t)(jnp.asarray(a)))
    def _A_setup():
        B, S, D, H = 1, 2048, 1024, 32
        Dh = D // H
        return {
            "x": _w((lambda *s: _rng.normal(s) * 0.05)(B, S, D)),
            "wq": _w((lambda *s: _rng.normal(s) * 0.2)(D, H * Dh)),
            "wk": _w((lambda *s: _rng.normal(s) * 0.2)(D, Dh)),
            "wv": _w((lambda *s: _rng.normal(s) * 0.05)(D, Dh)),
            "wo": _w((lambda *s: _rng.normal(s) * 0.05)(H * Dh, D)),
        }
    _A_in = _A_setup()

    def _B_setup():
        B, S, D, F = 1, 2048, 1024, 3584
        return {
            "x": _w((lambda *s: _rng.normal(s) * 0.05)(B, S, D)),
            "W_gate": _w((lambda *s: _rng.normal(s) * 0.8)(D, F) * (2.0 / D) ** 0.5),
            "W_up": _w((lambda *s: _rng.normal(s) * 0.8)(D, F) * (2.0 / D) ** 0.5),
            "W_down": _w((lambda *s: _rng.normal(s) * 0.8)(F, D) * (1.0 / F) ** 0.5),
        }
    _B_in = _B_setup()

    return {
        "A_x": _A_in["x"],
        "A_wq": _A_in["wq"],
        "A_wk": _A_in["wk"],
        "A_wv": _A_in["wv"],
        "A_wo": _A_in["wo"],
        "B_x": _B_in["x"],
        "B_W_gate": _B_in["W_gate"],
        "B_W_up": _B_in["W_up"],
        "B_W_down": _B_in["W_down"],
        "gate_w": _w((lambda *s: _rng.normal(s) * 0.05)(1024) * 16.0),
    }

def reference(A_x, A_wq, A_wk, A_wv, A_wo, B_x, B_W_gate, B_W_up, B_W_down, gate_w):
    def _A_ref(x, wq, wk, wv, wo):
        B, S, D = x.shape
        H = 32
        Dh = D // H
        q = (lambda x, *d: x.transpose(*d))((x @ wq).reshape(B, S, H, Dh), 0, 2, 1, 3)
        k = x @ wk
        v = x @ wv
        scores = jnp.einsum("bhqd,bkd->bhqk", q, k) * (Dh ** -0.5)
        p = _softmax(scores, axis=-1)
        o = jnp.einsum("bhqk,bkd->bhqd", p, v)
        return (lambda x, *d: x.transpose(*d))(o, 0, 2, 1, 3).reshape(B, S, H * Dh) @ wo

    def _B_ref(x, W_gate, W_up, W_down):
        gate = jnp.einsum("bsd,df->bsf", x, W_gate)
        up = jnp.einsum("bsd,df->bsf", x, W_up)
        gate = gate * (lambda x, dt: x.astype(dt))(gate > 0, gate.dtype)
        h = gate * up
        return jnp.einsum("bsf,fd->bsd", h, W_down)

    x = A_x
    g = _sigmoid((x * gate_w).sum(-1, keepdims=True))
    a = _A_ref(x, A_wq, A_wk, A_wv, A_wo)
    b = _B_ref(x, B_W_gate, B_W_up, B_W_down)
    return g * a + (1 - g) * b
```

```python
import functools
import math

import jax
import jax.numpy as jnp
from jax import lax
import jax.experimental.pallas as pl
import jax.experimental.pallas.tpu as pltpu

BF = jnp.bfloat16
F32 = jnp.float32
U32 = jnp.uint32
I32 = jnp.int32
NT = (((1,), (1,)), ((), ()))

S, D, H, DH, FF = 2048, 1024, 32, 32, 3584
T = 128
NKT = S // T
NG = D // T
NF = FF // T

CFG = dict(
    L=1,
    NCH=4,
    UNITS=16,
    GRP=2, OFF=-80, SHIFT=2,
    BUN=1,
    PH="ABCD",
)


def _a_combos(blk):
    n = len(blk)
    if n == 1:
        return [blk[0][0]]
    h = n // 2
    q = lambda i, j: [row[j * h:(j + 1) * h] for row in blk[i * h:(i + 1) * h]]
    a11, a12, a21, a22 = q(0, 0), q(0, 1), q(1, 0), q(1, 1)
    add = lambda x, y: [[u + v for u, v in zip(r, s)] for r, s in zip(x, y)]
    sub = lambda x, y: [[u - v for u, v in zip(r, s)] for r, s in zip(x, y)]
    ops = [add(a11, a22), add(a21, a22), a11, a22, add(a11, a12), sub(a21, a11), sub(a12, a22)]
    return [c for o in ops for c in _a_combos(o)]


def _strassen(leaf, b, idx=0):
    n = len(b)
    if n == 1:
        return [[leaf(idx, b[0][0])]]
    h = n // 2
    q = lambda i, j: [row[j * h:(j + 1) * h] for row in b[i * h:(i + 1) * h]]
    b11, b12, b21, b22 = q(0, 0), q(0, 1), q(1, 0), q(1, 1)
    badd = lambda x, y: [[u + v for u, v in zip(r, s)] for r, s in zip(x, y)]
    bsub = lambda x, y: [[u + [(-c, i) for c, i in v] for u, v in zip(r, s)] for r, s in zip(x, y)]
    add = lambda x, y: [[u + v for u, v in zip(r, s)] for r, s in zip(x, y)]
    sub = lambda x, y: [[u - v for u, v in zip(r, s)] for r, s in zip(x, y)]
    mul = lambda i, o: _strassen(leaf, o, idx * 7 + i)
    m2 = mul(1, b11)
    m4 = mul(3, bsub(b21, b11))
    c21 = add(m2, m4)
    m1 = mul(0, badd(b11, b22))
    t11 = add(m4, m1)
    t22 = sub(m1, m2)
    m3 = mul(2, bsub(b12, b22))
    t22 = add(t22, m3)
    m6 = mul(5, badd(b11, b12))
    c22 = add(t22, m6)
    m5 = mul(4, b22)
    c12 = add(m3, m5)
    t11 = sub(t11, m5)
    m7 = mul(6, badd(b21, b22))
    c11 = add(t11, m7)
    return [r + s for r, s in zip(c11, c12)] + [r + s for r, s in zip(c21, c22)]


def _rhs(comb, load):
    if len(comb) == 1 and comb[0][0] > 0:
        return load(comb[0][1])
    comb = sorted(comb, key=lambda t: -t[0])
    acc = load(comb[0][1]).astype(F32)
    if comb[0][0] < 0:
        acc = -acc
    for c, i in comb[1:]:
        v = load(i).astype(F32)
        acc = acc + v if c > 0 else acc - v
    return acc.astype(BF)


def _sum(xs):
    while len(xs) > 1:
        xs = [xs[i] + xs[i + 1] if i + 1 < len(xs) else xs[i] for i in range(0, len(xs), 2)]
    return xs[0]


def _ld(ref, *idx):
    return pltpu.bitcast(ref.bitcast(U32)[idx], BF)


def make_kernel(cfg):
    L = cfg["L"]
    NB = 2 ** L
    NP = 7 ** L
    RB = S // NB
    NCH = cfg["NCH"]
    RC = RB // NCH
    KX = NG // NB
    NQ = max(NG // NB, 1)
    GB = max(NB // 2, 1)
    NPAIR = NF // NB
    KO = NG // NB
    KD = KO + NPAIR
    ND = NG // NB
    UN = cfg["UNITS"]
    BUN = cfg["BUN"]
    scale = DH ** -0.5 * math.log2(math.e)
    ids = [[[(1, (i, j))] for j in range(NB)] for i in range(NB)]

    def kernel(x_hbm, wq_hbm, wkt_ref, wvt_ref, wo_hbm, wg_hbm, wu_hbm, wd_hbm, gw_ref, out_hbm,
               x_v, xa, wq_v, wg_v, wu_v, w2_v, qt, k_v, vt, g_v, o_v, ha, s0, s1, s2, s3, m_v, out_v,
               z_ref, sem_x, sem_wq, sem_w, sem_w2, sem_out):
        s_scr = (s0, s1, s2, s3)

        def cp_x(c):
            return pltpu.make_async_copy(x_hbm.at[:, pl.ds(c * RC, RC), :], x_v.at[c], sem_x.at[c])

        def cp_wq(j):
            return [pltpu.make_async_copy(wq_hbm.at[:, pl.ds((b * NQ + j) * T, T)], wq_v.at[j, b],
                                          sem_wq.at[j * NB + b]) for b in range(NB)]

        def cp_w(p):
            cols = pl.ds(pl.multiple_of(p * (NB * T), NB * T), NB * T)
            return [pltpu.make_async_copy(wg_hbm.at[:, cols], wg_v.at[p], sem_w.at[2 * p]),
                    pltpu.make_async_copy(wu_hbm.at[:, cols], wu_v.at[p], sem_w.at[2 * p + 1])]

        def cp_w2(j):
            r = []
            for b in range(NB):
                cols = pl.ds((b * ND + j) * T, T)
                r.append(pltpu.make_async_copy(wo_hbm.at[:, cols], w2_v.at[j, b, pl.ds(0, D)],
                                               sem_w2.at[2 * (j * NB + b)]))
                r.append(pltpu.make_async_copy(wd_hbm.at[:, cols], w2_v.at[j, b, pl.ds(D, FF)],
                                               sem_w2.at[2 * (j * NB + b) + 1]))
            return r

        def cp_out(j):
            r = []
            for b in range(NB):
                cols = pl.ds(pl.multiple_of((b * ND + j) * T, T), T)
                r.append(pltpu.make_async_copy(out_v.at[j, b], out_hbm.at[:, cols], sem_out.at[j * NB + b]))
            return r

        cp_x(0).start()
        for j in range(NQ):
            for c in cp_wq(j):
                c.start()
        for i in range(z_ref.shape[0]):
            z_ref[i] = 0

        gw = gw_ref[...].astype(F32)
        gw = jnp.concatenate([jnp.broadcast_to(gw[i:i + 1], (16, T)) for i in range(NG)], axis=1).astype(BF)
        wkv = jnp.concatenate([wkt_ref[...], wvt_ref[...], gw], axis=0)

        def phase_a(c, carry):
            @pl.when(c + 1 < NCH)
            def _():
                cp_x(c + 1).start()

            @pl.when(c == NCH - 1)
            def _():
                for cp in cp_w(0):
                    cp.start()

            cp_x(c).wait()

            @pl.when(c == 0)
            def _():
                for j in range(NQ):
                    for cp in cp_wq(j):
                        cp.wait()

            for rb in range(NB):
                for t in range(RC // T):
                    xt = x_v[c, rb, pl.ds(t * T, T), :]
                    kv = lax.dot_general(wkv, xt, NT, preferred_element_type=F32)
                    kt = rb * (RB // T) + c * (RC // T) + t
                    vt[kt] = kv[32:64].astype(BF)
                    kk = kv[0:32] * scale
                    k_v[kt] = jnp.concatenate([kk] * 4, axis=0).T.astype(BF)
                    g = jax.nn.sigmoid(kv[64:72])
                    g_v[kt] = jnp.concatenate([g] * 16, axis=0).T
            for k in range(KX):
                blk = [[x_v[c, i, :, pl.ds((j * KX + k) * T, T)].astype(F32) for j in range(NB)]
                       for i in range(NB)]
                for p, a in enumerate(_a_combos(blk)):
                    xa[c, p, k] = a.astype(BF)
            for j in range(NQ):
                def leaf(p, comb, j=j):
                    return _sum([jnp.dot(_ld(xa, c, p, k),
                                         _rhs(comb, lambda b: wq_v[j, b[1], pl.ds((b[0] * KX + k) * T, T), :]),
                                         preferred_element_type=F32) for k in range(KX)])
                cq = _strassen(leaf, ids)
                for rb in range(NB):
                    for b in range(NB):
                        for t in range(RC // T):
                            qb = rb * (RB // T) + c * (RC // T) + t
                            qt[qb, b * NQ + j] = cq[rb][b][t * T:(t + 1) * T].T.astype(BF)
            return carry

        lax.fori_loop(0, NCH, phase_a, 0)

        def phase_b(it, carry):
            for u in range(BUN):
                p0 = it * BUN + u
                @pl.when(p0 + BUN < NPAIR)
                def _():
                    for cp in cp_w(p0 + BUN):
                        cp.start()
            for u in range(BUN):
                for cp in cp_w(it * BUN + u):
                    cp.wait()
            for u in range(BUN):
                p0 = it * BUN + u
                hb = [[] for _ in range(NB)]
                for half in range(NB // GB):
                    def load(b, k, half=half):
                        w = (wg_v, wu_v)[b[1] % 2]
                        return w[p0, pl.ds((b[0] * KX + k) * T, T), pl.ds((half * GB + b[1] // 2) * T, T)]

                    def leaf(p, comb):
                        return _sum([jnp.dot(jnp.concatenate([_ld(xa, c, p, k) for c in range(NCH)], axis=0),
                                             _rhs(comb, functools.partial(load, k=k)),
                                             preferred_element_type=F32) for k in range(KX)])
                    if L == 0:
                        cc = [[leaf(0, [(1, (0, 0))]), leaf(0, [(1, (0, 1))])]]
                    else:
                        cc = _strassen(leaf, ids)
                    for rb in range(NB):
                        omg = 1.0 - g_v[pl.ds(rb * (RB // T), RB // T)].reshape(RB, T)
                        for i in range(GB):
                            hb[rb].append(jnp.maximum(cc[rb][2 * i], 0.0) * cc[rb][2 * i + 1] * omg)
                for p, a in enumerate(_a_combos(hb)):
                    ha[KO + p0, p] = a.astype(BF)
            return carry

        for u in range(1, BUN):
            for cp in cp_w(u):
                cp.start()
        if "B" in cfg["PH"]:
            lax.fori_loop(0, NPAIR // BUN, phase_b, 0)

        for j in range(ND):
            for cp in cp_w2(j):
                cp.start()

        n_it = NKT * H // UN
        GI = UN // 4

        class Ctx:
            def __init__(self):
                self.n = 0
                self.never = jnp.full((8, T), self.zero(), I32) != 0
                self.anchors = []

            def zero(self):
                self.n += 1
                return z_ref[self.n - 1]

        def qk_round(ctx, d, r):
            if r == 0:
                d["zk"] = ctx.zero()
                d["zs"] = ctx.zero()
                d["m"] = [None, None]
                d["cnt"] = 0
            vs = []
            for c in range(4 * r, 4 * r + 4):
                s = jnp.dot(_ld(k_v, d["zk"] + c)[:, :DH], d["q"], preferred_element_type=F32)
                d["buf"][d["zs"] + c] = s
                vs.append(s)
            for t in range(T // 8):
                for s in vs:
                    a = d["cnt"] % 2
                    d["cnt"] += 1
                    v = s[8 * t:8 * t + 8]
                    d["m"][a] = v if d["m"][a] is None else jnp.maximum(d["m"][a], v)
                    ctx.anchors.append(d["m"][a])
            if r == 3:
                m = jnp.max(jnp.maximum(d["m"][0], d["m"][1]), axis=0, keepdims=True)
                d["m"] = jnp.broadcast_to(m, (8, T))

        def pv_round(ctx, d, r, base, lo):
            if r == 0:
                d["zl"] = ctx.zero()
                d["zv"] = ctx.zero()
                d["l"] = None
                d["o"] = None
            m = d["m"]
            ps = [[] for _ in range(4)]
            cnt = 0
            for t in range(T // 16):
                for c4 in range(4):
                    if cnt % cfg["GRP"] == 0:
                        ai = base + 2 * cnt + cfg["OFF"]
                        m = d["m"]
                        if lo <= ai < len(ctx.anchors):
                            m = jnp.where(ctx.never, ctx.anchors[ai], m)
                    cnt += 1
                    s = d["buf"][d["zl"] + 4 * r + c4, pl.ds(16 * t, 16), :]
                    p0 = jnp.exp2(s[:8] - m)
                    p1 = jnp.exp2(s[8:] - m)
                    d["l"] = (p0 + p1) if d["l"] is None else d["l"] + (p0 + p1)
                    ps[c4] += [p0, p1]
            for c4 in range(4):
                p = jnp.concatenate(ps[c4], axis=0).astype(BF)
                o = jnp.dot(_ld(vt, d["zv"] + 4 * r + c4), p, preferred_element_type=F32)
                d["o"] = o if d["o"] is None else d["o"] + o
            if r == 3:
                d["o"] = d["o"] * (1.0 / jnp.sum(d["l"], axis=0, keepdims=True))

        def load_q(gi, h):
            return pltpu.bitcast(qt.bitcast(U32)[gi // NG, gi % NG, pl.ds(16 * h, 16), :], BF)

        ctx = Ctx()
        d0 = dict(q=load_q(0, 0), buf=s_scr[0])
        for r in range(4):
            qk_round(ctx, d0, r)
        m_v[...] = d0["m"]

        def phase_c(it, carry):
            ctx = Ctx()
            g0 = it * GI
            st = [dict(buf=s_scr[0], m=m_v[...])]
            for u in range(1, UN):
                st.append(dict(q=load_q(g0 + u // 4, u % 4), buf=s_scr[u % 4]))
            st.append(dict(q=load_q(jnp.minimum(g0 + GI, NKT * NG - 1), 0), buf=s_scr[0]))
            sh = cfg["SHIFT"] - 1
            for t in range(4 * UN + sh):
                if t < 4 * UN:
                    qk_round(ctx, st[1 + t // 4], t % 4)
                tt = t - sh
                if tt >= 0:
                    pv_round(ctx, st[tt // 4], tt % 4, 64 * t, 256 * (tt // 4))
            m_v[...] = st[UN]["m"]
            for a in range(GI):
                gi = g0 + a
                ot = jnp.concatenate([st[4 * a + h]["o"] for h in range(4)], axis=0)
                o_v[gi % NG, gi // NG] = ot.T * g_v[gi // NG]
            return carry

        if "C" in cfg["PH"]:
            lax.fori_loop(0, n_it, phase_c, 0)

        for j in range(ND):
            for cp in cp_w2(j):
                cp.wait()

        def o_combos(k, carry):
            blk = [[o_v[j * KO + k, pl.ds(i * (RB // T), RB // T)].reshape(RB, T) for j in range(NB)]
                   for i in range(NB)]
            for p, a in enumerate(_a_combos(blk)):
                ha[k, p] = a.astype(BF)
            return carry

        lax.fori_loop(0, KO, o_combos, 0)

        def phase_d(j, carry):
            def load(b, k):
                row = (b[0] * KO + k) if k < KO else (NG + (k - KO) * NB + b[0])
                return w2_v[j, b[1], pl.ds(row * T, T), :]

            def leaf(p, comb):
                acc = None
                for k0 in range(0, KD, 4):
                    r = _sum([jnp.dot(_ld(ha, k, p), _rhs(comb, functools.partial(load, k=k)),
                                      preferred_element_type=F32) for k in range(k0, min(k0 + 4, KD))])
                    acc = r if acc is None else acc + r
                return acc
            cc = _strassen(leaf, ids)
            for rb in range(NB):
                for b in range(NB):
                    out_v[j, b, pl.ds(rb * RB, RB), :] = cc[rb][b].astype(BF)
            for cp in cp_out(j):
                cp.start()
            return carry

        lax.fori_loop(0, ND, phase_d, 0)
        for j in range(ND):
            for cp in cp_out(j):
                cp.wait()

    scratch = [
        pltpu.VMEM((NCH, NB, RC, D), BF),
        pltpu.VMEM((NCH, NP, KX, RC, T), BF),
        pltpu.VMEM((NQ, NB, D, T), BF),
        pltpu.VMEM((NPAIR, D, NB * T), BF),
        pltpu.VMEM((NPAIR, D, NB * T), BF),
        pltpu.VMEM((ND, NB, D + FF, T), BF),
        pltpu.VMEM((NKT, NG, T, T), BF),
        pltpu.VMEM((NKT, T, T), BF),
        pltpu.VMEM((NKT, DH, T), BF),
        pltpu.VMEM((NKT, T, T), F32),
        pltpu.VMEM((NG, NKT, T, T), F32),
        pltpu.VMEM((KD, NP, RB, T), BF),
        pltpu.VMEM((NKT, T, T), F32),
        pltpu.VMEM((NKT, T, T), F32),
        pltpu.VMEM((NKT, T, T), F32),
        pltpu.VMEM((NKT, T, T), F32),
        pltpu.VMEM((8, T), F32),
        pltpu.VMEM((ND, NB, S, T), BF),
        pltpu.SMEM((4 * UN + 8,), I32),
        pltpu.SemaphoreType.DMA((NCH,)),
        pltpu.SemaphoreType.DMA((NQ * NB,)),
        pltpu.SemaphoreType.DMA((2 * NPAIR,)),
        pltpu.SemaphoreType.DMA((2 * ND * NB,)),
        pltpu.SemaphoreType.DMA((ND * NB,)),
    ]

    def run(A_x, A_wq, A_wk, A_wv, A_wo, B_x, B_W_gate, B_W_up, B_W_down, gate_w):
        del B_x
        hbm = pl.BlockSpec(memory_space=pl.ANY)
        vmem = pl.BlockSpec(memory_space=pltpu.VMEM)
        out = pl.pallas_call(
            kernel,
            out_shape=jax.ShapeDtypeStruct((S, D), BF),
            in_specs=[hbm, hbm, vmem, vmem, hbm, hbm, hbm, hbm, vmem],
            out_specs=hbm,
            scratch_shapes=scratch,
            compiler_params=pltpu.CompilerParams(
                vmem_limit_bytes=cfg.get("VMEM", 120) * 2 ** 20,
                disable_bounds_checks=cfg.get("NOBC", True),
                flags=cfg.get("FLAGS"),
            ),
            name="gated_mix",
        )(A_x.reshape(NB, RB, D), A_wq, A_wk.T, A_wv.T, A_wo, B_W_gate, B_W_up, B_W_down,
          gate_w.reshape(NG, T))
        return out.reshape(1, S, D)

    return run


@jax.jit
def pallas_gated_mix__grouped_kv_mqa__glu_gated_reglu__prompt_kernel(
    A_x: jax.Array,
    A_wq: jax.Array,
    A_wk: jax.Array,
    A_wv: jax.Array,
    A_wo: jax.Array,
    B_x: jax.Array,
    B_W_gate: jax.Array,
    B_W_up: jax.Array,
    B_W_down: jax.Array,
    gate_w: jax.Array,
):
    return make_kernel(CFG)(A_x, A_wq, A_wk, A_wv, A_wo, B_x, B_W_gate, B_W_up, B_W_down, gate_w)
```

```python
import bisect
import functools
import math

import jax
import jax.numpy as jnp
import numpy as np
from jax import lax
import jax.experimental.pallas as pl
import jax.experimental.pallas.tpu as pltpu

BF = jnp.bfloat16
F32 = jnp.float32
U32 = jnp.uint32
I32 = jnp.int32

S, D, DH, FF = 2048, 1024, 32, 3584
T = 128
NKT = S // T
NG = D // T
NGRP = NKT * NG

NB = 4
NP = 49
RB = S // NB
KX = NG // NB
NH = FF // T // NB
KD = KX + NH

VPU_ROUNDS = (1, 3)
AHEAD = [(0, 2), (1, 2), (2, 2), (3, 2), (2, 0), (3, 0)]
SPREAD = dict(x=24.0, wo=24.0, wd=24.0, q=16.0, h=64.0, w=2.0)
L_MIN, L_MAX = 2.0 ** -30, 2.0 ** 60

UNITS = 32
TIE = 2
C_STARTS = [-196, 132, 394, 689, 978, 1264, 1562, 1854]
B_START, B_END = -90, -150
B_SHARE = [3.54, 3.32, 3.26, 2.92, 2.39, 2.9, 1.48, 0.46, 3.16, 3.18, 2.79, 2.47, 2.84,
           3.13, 2.95, 3.04, 3.2, 1.21, 1.2, 2.66, 2.08, 2.24, 2.77, 3.39, 1.77, 0.47]
X_ROWS = 32
STAGES = [[3, (0, 1), (0, 0), (1, 0)], [2, (1, 1)], [1, 0, (1, 2), (1, 3), (0, 2), (0, 3)]]


def _quads(m):
    h = len(m) // 2
    return [[row[j * h:(j + 1) * h] for row in m[i * h:(i + 1) * h]] for i in range(2) for j in range(2)]


def _madd(x, y):
    return [[u + v for u, v in zip(r, s)] for r, s in zip(x, y)]


def _msub(x, y):
    return [[u + [(-c, i) for c, i in v] for u, v in zip(r, s)] for r, s in zip(x, y)]


def _add_terms(acc, terms):
    for sign, v in terms:
        acc = acc + v if sign > 0 else acc - v
    return acc


def _strassen(leaf, emit, early=False, a=None, b=None, idx=0, extra=lambda i, j: []):
    if a is None:
        a = b = [[[(1, (i, j))] for j in range(NB)] for i in range(NB)]
    if len(a) == 1:
        emit(0, 0, leaf(idx, a[0][0], b[0][0], *[extra(0, 0)] * early))
        return
    h = len(a) // 2
    a11, a12, a21, a22 = _quads(a)
    b11, b12, b21, b22 = _quads(b)
    m = {}

    def mul(i, x, y, block=None, terms=()):
        flip = i in (2, 5, 6, 7)
        col = lambda c: h - 1 - c if flip else c
        rest = lambda r, c: [(s, m[j, r, c]) for s, j in terms] + extra(block[0] * h + r, block[1] * h + c)
        inside = early and i > 5

        def keep(r, c, v):
            c = col(c)
            m[i, r, c] = v
            if block is not None:
                if not inside:
                    t = rest(r, c)
                    v = v + _add_terms(t[0][1], t[1:]) if h == 1 else _add_terms(v, t)
                emit(block[0] * h + r, block[1] * h + c, v)

        _strassen(leaf, keep, early, x, [r[::-1] for r in y] if flip else y, idx * 7 + i - 1,
                  lambda r, c: rest(r, col(c)) if inside else [])

    mul(2, _madd(a21, a22), b11)
    mul(4, a22, _msub(b21, b11), (1, 0), [(1, 2)])
    mul(1, _madd(a11, a22), _madd(b11, b22))
    mul(3, a11, _msub(b12, b22))
    mul(6, _msub(a21, a11), _madd(b11, b12), (1, 1), [(1, 1), (-1, 2), (1, 3)])
    mul(5, _madd(a11, a12), b22, (0, 1), [(1, 3)])
    mul(7, _msub(a12, a22), _madd(b21, b22), (0, 0), [(1, 4), (1, 1), (-1, 5)] if h == 1 else [(1, 1), (1, 4), (-1, 5)])


def _lin(terms, load):
    if len(terms) == 1:
        assert terms[0][0] > 0
        return load(terms[0][1]).astype(BF)

    def pair(u, v):
        if u[0] == v[0]:
            return u[0], u[1] + v[1]
        return (1, u[1] - v[1]) if u[0] > 0 else (1, v[1] - u[1])

    vals = [(c, load(i).astype(F32)) for c, i in terms]
    while len(vals) > 1:
        vals = [pair(vals[i], vals[i + 1]) for i in range(0, len(vals), 2)]
    assert vals[0][0] > 0
    return vals[0][1].astype(BF)


def _sum(xs):
    while len(xs) > 1:
        xs = [xs[i] + xs[i + 1] if i + 1 < len(xs) else xs[i] for i in range(0, len(xs), 2)]
    return xs[0]


def _fold(x):
    return jnp.sum(x.reshape(-1, 8, T), axis=0)


def _flip(x):
    return jnp.concatenate([x[i:i + 16] for i in range(x.shape[0] - 16, -1, -16)], axis=0)


def _ld(ref, *idx):
    return pltpu.bitcast(ref.bitcast(U32)[idx], BF)


def _dot(a, b):
    return jnp.dot(a, b, preferred_element_type=F32)


def _grp(g):
    return NKT - 1 - g // NG, g % NG


def _mxu_rows(h, r):
    return T - 16 * (r in VPU_ROUNDS or (h, r) in AHEAD)


class _Pace:
    def __init__(self, z_ref):
        self.z_ref, self.used, self.times, self.vals = z_ref, 0, [], []
        self.never = jnp.full((8, T), self.zero(), I32) != 0

    def zero(self):
        self.used += 1
        return self.z_ref[self.used - 1]

    def mark(self, t, x, row):
        i = bisect.bisect_right(self.times, t)
        self.times.insert(i, t)
        self.vals.insert(i, (x, row))

    def after(self, t, x):
        i = bisect.bisect_right(self.times, t) - 1
        if i < 0:
            return x
        y, row = self.vals[i]
        return jnp.where(self.never, y[row:row + 8, :T], x)


def _kernel(x_hbm, wq_hbm, wkt_hbm, wvt_hbm, wo_hbm, wg_hbm, wu_hbm, wd_hbm, gw_hbm, out_hbm,
            x_v, xa, wq_v, wg_v, wu_v, w2_v, qt, k_v, vt, g_v, omg_v, hf, kb, pp_v, lp_v, pc_v,
            oc_v, out_v, wkv_v, gw_v, lc_v, z_ref, sem_in, sem_w, sem_w2, sem_out):
    def cp_stage(s):
        cps = [pltpu.make_async_copy(x_hbm.at[v], x_v.at[v], sem_in.at[s]) if isinstance(v, int) else
               pltpu.make_async_copy(wq_hbm.at[pl.ds(v[0] * D // 2, D // 2), pl.ds(v[1] * KX * T, KX * T)],
                                     wq_v.at[v], sem_in.at[s]) for v in STAGES[s]]
        if s == 0:
            cps += [pltpu.make_async_copy(wkt_hbm, wkv_v.at[pl.ds(0, DH)], sem_in.at[0]),
                    pltpu.make_async_copy(wvt_hbm, wkv_v.at[pl.ds(DH, DH)], sem_in.at[0]),
                    pltpu.make_async_copy(gw_hbm, gw_v, sem_in.at[0])]
        return cps

    def cp_w(i):
        cols = pl.ds(pl.multiple_of(i * (2 * T), 2 * T), 2 * T)
        return [pltpu.make_async_copy(wg_hbm.at[:, cols], wg_v.at[i % 2], sem_w.at[i % 2]),
                pltpu.make_async_copy(wu_hbm.at[:, cols], wu_v.at[i % 2], sem_w.at[i % 2])]

    cp_w2 = [pltpu.make_async_copy(wo_hbm, w2_v.at[pl.ds(0, D)], sem_w2),
             pltpu.make_async_copy(wd_hbm, w2_v.at[pl.ds(D, FF)], sem_w2)]

    def cp_out(rb, b):
        return pltpu.make_async_copy(
            out_v.at[rb, b],
            out_hbm.at[pl.ds(pl.multiple_of(rb * RB, RB), RB), pl.ds(pl.multiple_of(b * KX * T, KX * T), KX * T)],
            sem_out)

    def clear(i, carry):
        z_ref[i] = 0
        return carry

    queue = [cp_stage(s) for s in range(len(STAGES))] + [cp_w(0)]
    for i, cps in enumerate(queue):
        for cp in cps:
            cp.start()
        lax.fori_loop(2 * i, 2 * i + 2 if i + 1 < len(queue) else z_ref.shape[0], clear, 0)

    def load_q(qb, hg, h):
        return _ld(qt, qb, hg, pl.ds(16 * h, 16))

    def vpu_probs(pace, qb, hg, h, r, when, rows):
        z = pace.zero()
        if not rows:
            q = load_q(z + qb, hg, h).astype(F32)
            rows += [jnp.broadcast_to(q[f:f + 1], (8, T)) for f in range(DH)]
        acc = None
        for f in range(DH):
            q = pace.after(when(f / DH), rows[f]) if f % TIE == 0 else rows[f]
            v = kb[z + r, f] * jnp.concatenate([q] * 8, axis=0)
            acc = v if acc is None else acc + v
        return jnp.exp2(acc)

    def add_sum(d, v):
        d["l"] = v if d["l"] is None else d["l"] + v

    def prepend(d, r, p):
        d[r] = [jnp.concatenate([p[16 * c:16 * c + 16], d[r][c]], axis=0) for c in range(4)]

    def qk_round(pace, d, r, t0):
        rows = _mxu_rows(d["h"], r)
        ss = [_dot(_ld(k_v, d["z"], 4 * r + c, pl.ds(0, rows // 2))[:, :DH], d["q"]) for c in range(4)]
        for t in range(0, rows, 16):
            for c in range(4):
                pace.mark(t0 + t + 4 * c, ss[c], t)
        ps = [jnp.exp2(s) for s in ss]
        add_sum(d, _fold(_sum(ps)))
        d[r] = [_flip(p) for p in ps]
        return rows

    def pv_round(pace, d, r, ps, t0):
        z = pace.zero()
        outs = [_dot(_ld(vt, z, 4 * r + c), ps[c]) for c in range(4)]
        for t in range(0, DH, 8):
            for c in (0, 2):
                pace.mark(t0 + t + 2 * c, outs[c], t)
        d["o"] = _sum(outs) if r == 0 else d["o"] + _sum(outs)

    def hand_over(d):
        for c in range(4):
            pc_v[c] = d[0][c].astype(BF)
        lc_v[...] = d["l"]

    def put_o(qb, hg, ot):
        rows = pl.ds(pl.multiple_of(qb % (RB // T) * T, T), T)
        hf[hg % KX, hg // KX, qb // (RB // T), rows, :] = ot.T * g_v[qb]

    k16 = {}

    def kv_proj(rb):
        for t in range(RB // T):
            kv = lax.dot_general(wkv_v[...], x_v[rb, pl.ds(t * T, T), :], (((1,), (1,)), ((), ())),
                                 preferred_element_type=F32)
            kt = rb * (RB // T) + t
            vt[0, kt] = kv[DH:2 * DH].astype(BF)
            k = jnp.concatenate([kv[:DH] * (DH ** -0.5 * math.log2(math.e))] * 4, axis=0).T
            k_v[0, kt] = _flip(k).astype(BF)
            k16[kt] = k[:16]
            g = jnp.concatenate([jax.nn.sigmoid(kv[2 * DH:2 * DH + 8])] * 16, axis=0).T
            g_v[kt] = g
            omg_v[rb, pl.ds(t * T, T), :] = 1.0 - g

    def project():
        todo, here = [], []
        _strassen(lambda *prod: todo.append(prod) or 0.0, lambda *_: None)
        never = jnp.full((8, T), z_ref[0], I32) != 0
        nq = KX * RB // X_ROWS

        def x_sums(prods, i, z, after=None):
            k, rows = i // (RB // X_ROWS), pl.ds(i % (RB // X_ROWS) * X_ROWS, X_ROWS)
            src = {}
            for _, ta, _ in prods:
                for _, b in ta:
                    if b not in src:
                        v = x_v[z + b[0], rows, pl.ds((b[1] * KX + k) * T, T)].astype(F32).reshape(-1, 8, T)
                        src[b] = (v if after is None else jnp.where(never, after, v)).reshape(X_ROWS, T)
            for p, ta, _ in prods:
                xa[p, k, rows, :] = _lin(ta, src.get)

        for s, stage in enumerate(STAGES):
            for cp in cp_stage(s):
                cp.wait()
            if s == 0:
                gw = gw_v[...].astype(F32)
                wkv_v[pl.ds(2 * DH, 16), :] = jnp.concatenate(
                    [jnp.broadcast_to(gw[i:i + 1], (16, T)) for i in range(NG)], axis=1).astype(BF)
            for v in stage:
                if isinstance(v, int):
                    kv_proj(v)
            here += stage
            run = [v for v in todo if all(b[0] in here for _, b in v[1])
                   and all((b[0] // 2, b[1]) in here for _, b in v[2])]
            todo = [v for v in todo if v not in run]
            i, jobs = 2, []
            for q in range(nq):
                x_sums(run[:i], q, z_ref[1])
            while i < len(run):
                j = i + 1
                while j < len(run) and run[j][0] // 7 == run[i][0] // 7:
                    j += 1
                lo = max(jobs[-1][2] if jobs else 0, i - 9)
                jobs.append((run[i:j], lo, max(lo + 1, min(i - 1, lo + 4)), z_ref[2 + i]))
                i = j
            for n, (p, ta, tb) in enumerate(run):
                res = _sum([_dot(_ld(xa, p, k), _lin(
                    tb, lambda b: wq_v[b[0] // 2, b[1], pl.ds((b[0] % 2 * KX + k) * T, T), :])) for k in range(KX)])
                for prods, n0, n1, z in jobs:
                    if n0 <= n < n1:
                        q0, q1 = (n - n0) * nq // (n1 - n0), (n + 1 - n0) * nq // (n1 - n0)
                        for q in range(q0, q1):
                            t = (q - q0) * (RB // 8) // (q1 - q0) * 8
                            x_sums(prods, q, z, res[t:t + 8, :T])
                if not todo and n == 4:
                    for kt in range(NKT):
                        for f in range(DH):
                            kb[kt // 4, f, pl.ds(kt % 4 * 16, 16), :] = jnp.broadcast_to(k16[kt][:, f:f + 1], (16, T))
                yield p, res

    done, products = {}, project()

    def q_leaf(p, ta, tb):
        while p not in done:
            done.update([next(products)])
        return done[p]

    def q_emit(rb, b, v):
        for j in range(KX):
            for t in range(RB // T):
                qt[rb * (RB // T) + t, b * KX + j] = v[t * T:(t + 1) * T, j * T:(j + 1) * T].T.astype(BF)

    _strassen(q_leaf, q_emit)

    first = dict(h=0, z=0, l=None, q=load_q(*_grp(0), 0))
    qk_round(_Pace(z_ref), first, 0, 0)
    hand_over(first)
    oc_v[...] = jnp.zeros_like(oc_v)

    n_ahead = NGRP * len(AHEAD)
    per_it = -(-n_ahead // (2 * NH))
    knots = [B_START] + [RB * i for i in range(NP // 2 + 1)] + [NP * RB // 2 + B_END]
    share = np.cumsum([0.0] + [f * (t1 - t0) for f, t0, t1 in zip(B_SHARE, knots, knots[1:])])
    due = lambda i: float(np.interp(i / per_it * share[-1], share, knots))

    def phase_b(it, carry):
        @pl.when(it + 1 < 2 * NH)
        def _():
            for cp in cp_w(it + 1):
                cp.start()
        for cp in cp_w(it):
            cp.wait()
        pace, todo = _Pace(z_ref), list(range(per_it))
        stores, tiles, got, ran = [], {}, {}, []

        def catch_up(now):
            while todo and due(todo[0] + 1) <= now:
                i = todo.pop(0)
                n = jnp.minimum(it * per_it + i, n_ahead - 1)
                g, j = n // len(AHEAD), n % len(AHEAD)
                h, r = jnp.where(j < 4, j, j - 2), jnp.where(j < 4, 2, 0)
                p = vpu_probs(pace, *_grp(g), h, r, lambda x: due(i + x), [])
                stores.append((due(i + 1), pp_v, n, p.astype(BF)))
                stores.append((due(i + 1), lp_v, n, _sum([p[t:t + 8] for t in range(0, 64, 8)])))
            stores.sort(key=lambda s: s[0])
            while stores and stores[0][0] <= now:
                _, ref, idx, v = stores.pop(0)
                ref[idx] = v

        def load(b, k, wide):
            if (b, k, wide) not in tiles:
                w = (wg_v, wu_v)[b[1] % 2][it % 2, pl.ds((b[0] * KX + k) * T, T), pl.ds(b[1] // 2 * T, T)]
                tiles[b, k, wide] = w.astype(F32) if wide else w
            return tiles[b, k, wide]

        def leaf(p, ta, tb):
            n = len(ran)
            ran.append(p)
            ws = [_lin(tb, functools.partial(load, k=k, wide=len(tb) > 1)) for k in range(KX)]
            if n % 2 == 0:
                catch_up(n // 2 * RB)
            rows = RB // 2 if n == NP - 1 else RB
            vs = [_sum([_dot(_ld(xa, p, k, pl.ds(i // 2, rows // 2)), ws[k]) for k in range(KX)])
                  for i in range(0, RB, rows)]
            if n % 2 == 0:
                for t in range(0, rows, 8):
                    pace.mark(n // 2 * RB + t, vs[0], t)
            return jnp.concatenate(vs, axis=0)

        def emit(rb, b, v):
            got[rb, b] = v
            if (rb, b ^ 1) in got:
                stores.append(((len(ran) + 1) // 2 * RB, hf, (KX + it // 2, it % 2 * 2 + b // 2, rb),
                               jnp.maximum(got[rb, b & ~1], 0.0) * got[rb, b | 1] * omg_v[rb]))

        _strassen(leaf, emit)
        catch_up(math.inf)
        return carry

    lax.fori_loop(0, 2 * NH, phase_b, 0)

    for cp in cp_w2:
        cp.start()
    period = sum(_mxu_rows(h, r) + DH for h in range(4) for r in range(4))
    starts = C_STARTS + [C_STARTS[0] + period]

    def phase_c(it, bad):
        pace, g0 = _Pace(z_ref), it * (UNITS // 4)
        put_o(*_grp(jnp.maximum(g0 - 1, 0)), oc_v[...])
        units = []
        for u in range(UNITS + 1):
            g = jnp.minimum(g0 + u // 4, NGRP - 1)
            units.append(dict(g=g, h=u % 4, z=pace.zero(), l=None, q=load_q(*_grp(g), u % 4), rows=[]))
        units[0]["l"] = lc_v[...]
        t = n_vpu = 0
        for i in range(4 * UNITS):
            d, r = units[(i + 1) // 4], (i + 1) % 4
            t += qk_round(pace, d, r, t)
            if r in VPU_ROUNDS:
                a, b = divmod(n_vpu, len(starts) - 1)
                when = lambda x: a * period + starts[b] + x * (starts[b + 1] - starts[b])
                p = vpu_probs(pace, *_grp(d["g"]), d["h"], r, when, d["rows"])
                n_vpu += 1
                add_sum(d, _sum([p[j:j + 8] for j in range(0, 64, 8)]))
                prepend(d, r, p)
            d, r = units[i // 4], i % 4
            if (d["h"], r) in AHEAD:
                n = d["g"] * len(AHEAD) + AHEAD.index((d["h"], r))
                add_sum(d, lp_v[n])
                prepend(d, r, pp_v[n].astype(F32))
            pv_round(pace, d, r, [_ld(pc_v, c) if i == 0 else d[r][c].astype(BF) for c in range(4)], t)
            t += DH
            if r == 3:
                l = jnp.sum(d["l"], axis=0, keepdims=True)
                d["o"] = d["o"] * (1.0 / l)
                bad = jnp.where((l > L_MIN) & (l < L_MAX) & (_fold(d["o"]) * 0.0 == 0.0), bad, 1.0)
        hand_over(units[UNITS])
        for u in range(0, UNITS, 4):
            ot = jnp.concatenate([d["o"] for d in units[u:u + 4]], axis=0)
            if u + 4 < UNITS:
                put_o(*_grp(units[u]["g"]), ot)
            else:
                oc_v[...] = ot
        return bad

    bad = lax.fori_loop(0, 4 * NGRP // UNITS, phase_c, jnp.zeros((8, T), F32))

    for cp in cp_w2:
        cp.wait()
    last_o = oc_v[...]

    never = jnp.full((1, 8, T), z_ref[0], I32) != 0
    total, peak = {}, {}

    def job(key, load):
        def run(after):
            vs = load()
            n = vs[0].shape[0]
            vs = [jnp.abs(jnp.where(never, after[i * n % RB:i * n % RB + n, :T].reshape(-1, 8, T),
                                    v.astype(F32).reshape(-1, 8, T))) for i, v in enumerate(vs)]
            v, top = _sum(vs), functools.reduce(jnp.maximum, vs)
            if key == "q":
                v = top = jnp.broadcast_to(jnp.sum(v, axis=2, keepdims=True), v.shape)
            total[key] = total.get(key, 0.0) + jnp.sum(v, axis=0)
            peak[key] = jnp.maximum(peak.get(key, 0.0), jnp.max(top, axis=0))
        return run

    jobs = [job("x", lambda rb=rb, j=j: [x_v[rb, :, pl.ds(j * T, T)]]) for rb in range(NB) for j in range(NG)]
    jobs += [job("wo" if r < D else "wd", lambda r=r, j=j: [w2_v[pl.ds(r, RB), pl.ds((j + i) * T, T)] for i in range(2)])
             for r in range(0, D + FF, RB) for j in range(0, NG, 2)]
    jobs += [job("q", lambda hg=hg: [qt[qb, hg] for qb in range(0, NKT, 4)]) for hg in range(NG)]
    jobs += [job(("h", k, cb), lambda k=k, cb=cb: [hf[k, cb, rb, pl.ds(0, T), :] for rb in range(NB)])
             for k in range(KX, KD) for cb in range(NB)]
    jobs += [job(i, lambda w=w: [w[0, pl.ds(0, T), pl.ds(j * T, T)] for j in range(2)])
             for i, w in enumerate((wg_v, wu_v))]

    def checks_pass():
        ok = jnp.max(bad) == 0.0
        for key, n in (("x", S * D), ("wo", D * D), ("wd", FF * D), ("q", D * T)):
            ok &= jnp.max(peak[key]) <= SPREAD[key] / n * jnp.sum(total[key])
        cols = [jnp.sum(v, axis=0, keepdims=True) for key, v in total.items() if isinstance(key, tuple)]
        ok &= jnp.max(functools.reduce(jnp.maximum, cols)) <= SPREAD["h"] / FF * jnp.sum(_sum(cols))
        gate, up = jnp.sum(total[0]), jnp.sum(total[1])
        return ok & (gate <= SPREAD["w"] * up) & (up <= SPREAD["w"] * gate)

    trust = []
    n_dot, tiles = [0], {}

    def out_leaf(p, ta, tb, extra):
        def load(b, k):
            key = (p // 7, b, k, len(tb) > 1)
            if key not in tiles:
                row = b[0] * KX + k if k < KX else NG + (k - KX) * NB + b[0]
                w = w2_v[pl.ds(row * T, T), pl.ds(b[1] * KX * T, KX * T)]
                tiles[key] = w.astype(F32) if len(tb) > 1 else w
            return tiles[key]

        z, acc, pend, i = z_ref[p], [], [], 0
        for k in list(range(KX, KD)) + list(range(KX)):
            pend.append(_dot(_lin(ta, lambda b: hf[z + k, b[1], b[0]]), _lin(tb, functools.partial(load, k=k))))
            n_dot[0] += 1
            if n_dot[0] == NH - 1:
                put_o(*_grp(NGRP - 1), last_o)
            if jobs and n_dot[0] % 2 == 0 and n_dot[0] > KD and p // 7 in (1, 0, 2, 4):
                jobs.pop(0)(pend[-1])
                if not jobs:
                    trust.append(checks_pass())
            if n_dot[0] % 2 == 0 or k == KX - 1:
                acc, pend, i = [_add_terms(_sum([_sum(pend)] + acc), extra[i::3] if i < 3 else [])], [], i + 1
        return acc[0]

    def out_emit(rb, b, v):
        out_v[rb, b] = v.astype(BF)
        cp_out(rb, b).start()

    _strassen(out_leaf, out_emit, early=True)
    for rb in range(NB):
        for b in range(NB):
            cp_out(rb, b).wait()

    @pl.when(jnp.logical_not(trust[0]))
    def _():
        def q_block(n, carry):
            qb, b = n // NB, n % NB
            x = x_v[qb // (RB // T), pl.ds(pl.multiple_of(qb % (RB // T) * T, T), T), :]
            q = _dot(x[:, :D // 2], wq_v[0, b]) + _dot(x[:, D // 2:], wq_v[1, b])
            for j in range(KX):
                qt[qb, b * KX + j] = q[:, j * T:(j + 1) * T].T.astype(BF)
            return carry

        def h_block(n, carry):
            i, rb = n // NB, n % NB

            @pl.when(rb == 0)
            def _():
                for cp in cp_w(i):
                    cp.start()
                for cp in cp_w(i):
                    cp.wait()

            h = jnp.maximum(_dot(x_v[rb], wg_v[i % 2]), 0.0) * _dot(x_v[rb], wu_v[i % 2])
            for j in range(2):
                hf[KX + i // 2, i % 2 * 2 + j, rb] = h[:, j * T:(j + 1) * T] * omg_v[rb]
            return carry

        def unit(u, carry):
            (qb, hg), h = _grp(u // 4), u % 4
            q = _ld(qt, qb, hg, pl.ds(pl.multiple_of(16 * h, 16), 16))
            ss = [_dot(_ld(k_v, 0, c)[:, :DH], q) for c in range(NKT)]
            m = jnp.max(functools.reduce(jnp.maximum, ss), axis=0, keepdims=True)
            ps = [jnp.exp2(s - m) for s in ss]
            l = jnp.sum(_sum(ps), axis=0, keepdims=True)
            o = _sum([_dot(_ld(vt, 0, c), _flip(p).astype(BF)) for c, p in enumerate(ps)])
            oc_v[pl.ds(pl.multiple_of(DH * h, DH), DH), :] = o * (1.0 / l)

            @pl.when(h == 3)
            def _():
                put_o(qb, hg, oc_v[...])
            return carry

        def block(n, carry):
            rb, b = n // NB, n % NB
            cols = pl.ds(pl.multiple_of(b * KX * T, KX * T), KX * T)

            def step(k, acc):
                for cb in range(NB):
                    row = jnp.where(k < KX, cb * KX + k, NG + (k - KX) * NB + cb) * T
                    acc += _dot(hf[k, cb, rb].astype(BF), w2_v[pl.ds(pl.multiple_of(row, T), T), cols])
                return acc

            out_v[rb, b] = lax.fori_loop(0, KD, step, jnp.zeros((RB, KX * T), F32)).astype(BF)
            cp_out(rb, b).start()
            cp_out(rb, b).wait()
            return carry

        lax.fori_loop(0, NKT * NB, q_block, 0)
        lax.fori_loop(0, 2 * NH * NB, h_block, 0)
        lax.fori_loop(0, 4 * NGRP, unit, 0)
        lax.fori_loop(0, NB * NB, block, 0)


@jax.jit
def pallas_gated_mix__grouped_kv_mqa__glu_gated_reglu__prompt_kernel(
    A_x: jax.Array,
    A_wq: jax.Array,
    A_wk: jax.Array,
    A_wv: jax.Array,
    A_wo: jax.Array,
    B_x: jax.Array,
    B_W_gate: jax.Array,
    B_W_up: jax.Array,
    B_W_down: jax.Array,
    gate_w: jax.Array,
):
    del B_x
    vmem, dma = pltpu.VMEM, pltpu.SemaphoreType.DMA
    scratch = [
        vmem((NB, RB, D), BF),
        vmem((NP, KX, RB, T), BF),
        vmem((2, NB, D // 2, KX * T), BF),
        vmem((2, D, 2 * T), BF),
        vmem((2, D, 2 * T), BF),
        vmem((D + FF, D), BF),
        vmem((NKT, NG, T, T), BF),
        vmem((1, NKT, T, T), BF),
        vmem((1, NKT, DH, T), BF),
        vmem((NKT, T, T), F32),
        vmem((NB, RB, T), F32),
        vmem((KD, NB, NB, RB, T), F32),
        vmem((4, DH, 64, T), F32),
        vmem((NGRP * len(AHEAD), 64, T), BF),
        vmem((NGRP * len(AHEAD), 8, T), F32),
        vmem((4, T, T), BF),
        vmem((T, T), F32),
        vmem((NB, NB, RB, KX * T), BF),
        vmem((2 * DH + 16, D), BF),
        vmem((NG, T), BF),
        vmem((8, T), F32),
        pltpu.SMEM((max(7 * UNITS + 8, 64),), I32),
        dma((len(STAGES),)), dma((2,)), dma(()), dma(()),
    ]

    hbm = pl.BlockSpec(memory_space=pl.ANY)
    out = pl.pallas_call(
        _kernel,
        out_shape=jax.ShapeDtypeStruct((S, D), BF),
        in_specs=[hbm] * 9,
        out_specs=hbm,
        scratch_shapes=scratch,
        compiler_params=pltpu.CompilerParams(vmem_limit_bytes=124 * 2 ** 20, disable_bounds_checks=True),
        name="gated_mix",
    )(A_x.reshape(NB, RB, D), A_wq, A_wk.T, A_wv.T, A_wo, B_W_gate, B_W_up, B_W_down,
      gate_w.reshape(NG, T))
    return out.reshape(1, S, D)
```
